```python
import jax
import jax.numpy as jnp

def _softmax(x, axis=-1):
    return jax.nn.softmax(x, axis=axis)

def _gelu(x):
    return jax.nn.gelu(x, approximate=True)

def _silu(x):
    return jax.nn.silu(x)

def _sigmoid(x):
    return jax.nn.sigmoid(x)

def _layernorm(x, axis=-1, eps=1e-05):
    m = jnp.mean(x, axis=axis, keepdims=True)
    v = jnp.var(x, axis=axis, keepdims=True)
    return (x - m) / jnp.sqrt(v + eps)

def _scatter_add(tgt, idx, src, axis=0):
    return tgt.at[idx].add(src)

def _segment_sum(src, seg, n):
    return jax.ops.segment_sum(src, seg, n)

class _Rng:

    def __init__(self, key):
        self._k = key

    def _next(self):
        self._k, sub = jax.random.split(self._k)
        return sub

    def normal(self, shape):
        return jax.random.normal(self._next(), shape, dtype=jnp.bfloat16)

    def randint(self, lo, hi, shape):
        return jax.random.randint(self._next(), shape, lo, hi, dtype=jnp.int32)

    def uniform(self, shape, lo=0.0, hi=1.0):
        return jax.random.uniform(self._next(), shape, jnp.bfloat16, lo, hi)

    def permutation(self, n):
        return jax.random.permutation(self._next(), n)
kernel_name = 'adaLN_cond__ssm_conv_h3__glu_gated_bilinear__prompt'

def setup_inputs():
    _rng = _Rng(jax.random.key(int.from_bytes(__import__("os").urandom(4), "little")))
    _w = lambda a: (lambda t: t.astype(jnp.bfloat16) if jnp.issubdtype(t.dtype, jnp.floating) else t)(jnp.asarray(a))

    def _A_setup():
        B, S, D = (1, 2048, 640)
        ks = 4
        return {'q': _w((lambda *s: _rng.normal(s) * 0.05)(B, S, D)), 'k': _w((lambda *s: _rng.normal(s) * 0.05)(B, S, D)), 'v': _w((lambda *s: _rng.normal(s) * 0.05)(B, S, D)), 'shift_k': _w((lambda *s: _rng.normal(s) * 0.05)(D, ks) * 0.5), 'ssm_k': _w((lambda *s: _rng.normal(s) * 0.05)(D, S) * (1.0 / S ** 0.5)), 'ssm_D': _w((lambda *s: _rng.normal(s) * 0.05)(D))}
    _A_in = _A_setup()

    def _B_setup():
        B, S, D, F = (1, 2048, 640, 1536)
        return {'x': _w((lambda *s: _rng.normal(s) * 0.05)(B, S, D)), 'w_gate': _w((lambda *s: _rng.normal(s) * 0.05)(D, F) * D ** (-0.5)), 'w_up': _w((lambda *s: _rng.normal(s) * 0.05)(D, F) * D ** (-0.5)), 'w_down': _w((lambda *s: _rng.normal(s) * 0.05)(F, D) * F ** (-0.5))}
    _B_in = _B_setup()
    return {'A_q': _A_in['q'], 'A_k': _A_in['k'], 'A_v': _A_in['v'], 'A_shift_k': _A_in['shift_k'], 'A_ssm_k': _A_in['ssm_k'], 'A_ssm_D': _A_in['ssm_D'], 'B_x': _B_in['x'], 'B_w_gate': _B_in['w_gate'], 'B_w_up': _B_in['w_up'], 'B_w_down': _B_in['w_down'], 'c': _w((lambda *s: _rng.normal(s) * 0.05)(1, 640)), 'w_mod': _w((lambda *s: _rng.normal(s) * 0.05)(640, 6 * 640) * 640 ** (-0.5))}

def reference(A_q, A_k, A_v, A_shift_k, A_ssm_k, A_ssm_D, B_x, B_w_gate, B_w_up, B_w_down, c, w_mod):

    def _A_ref(q, k, v, shift_k, ssm_k, ssm_D):
        B, S, D = q.shape
        ks = shift_k.shape[-1]
        k_pad = jnp.pad(k, ((0, 0), (ks - 1, 0), (0, 0)))
        k_shift = jnp.zeros_like(k)
        for t in range(ks):
            k_shift = k_shift + k_pad[:, t:t + S, :] * shift_k[:, ks - 1 - t][None, None, :]
        kv = k_shift * v
        L = 2 * S
        kv_pad = jnp.pad(kv, ((0, 0), (0, S), (0, 0)))
        kf_pad = jnp.pad(ssm_k, ((0, 0), (0, S)))
        kv_f = (lambda x, axes=(-2, -1): jnp.fft.rfft2(x.astype(jnp.float32), axes=axes))(kv_pad[:, None, :, :], axes=(1, 2))
        kf_f = (lambda x, axes=(-2, -1): jnp.fft.rfft2(x.astype(jnp.float32), axes=axes))(kf_pad[:, None, :], axes=(1, 2))
        kf_f = (lambda x, *d: x.transpose(*d))(kf_f, 1, 2, 0)
        y_f = kv_f * kf_f[None, :, :, :]
        y = (lambda x, s, axes=(-2, -1): jnp.fft.irfft2(x, s=s, axes=axes).astype(jnp.bfloat16))(y_f, (1, L), axes=(1, 2))[:, 0, :S, :]
        y = y + kv * ssm_D[None, None, :]
        return q * y

    def _B_ref(x, w_gate, w_up, w_down):
        g = jnp.einsum('bsd,df->bsf', x, w_gate)
        u = jnp.einsum('bsd,df->bsf', x, w_up)
        h = g * u
        return jnp.einsum('bsf,fd->bsd', h, w_down)
    x = A_q
    mod = (_silu(c) @ w_mod).reshape(c.shape[0], 6, 1, -1)
    sa, ca, ga, sb, cb, gb = (mod[:, 0].copy(), mod[:, 1].copy(), mod[:, 2].copy(), mod[:, 3].copy(), mod[:, 4].copy(), mod[:, 5].copy())
    h = _layernorm(x, axis=-1) * (1 + ca) + sa
    x = x + ga * _A_ref(h, A_k, A_v, A_shift_k, A_ssm_k, A_ssm_D)
    h = _layernorm(x, axis=-1) * (1 + cb) + sb
    x = x + gb * _B_ref(h, B_w_gate, B_w_up, B_w_down)
    return x
```

```python
import numpy as np
import jax
import jax.numpy as jnp
from jax import lax
import jax.experimental.pallas as pl
import jax.experimental.pallas.tpu as pltpu

S, D, F = 2048, 640, 1536
T = 128
NB = S // T
CT = D // 128
BM = 256
NSTEP = S // BM
EPS = 1e-5
BF = jnp.bfloat16
F32 = jnp.float32


def _dft_matrices():
    f = np.concatenate([np.arange(0, T, 2), np.arange(1, T, 2)]).astype(np.float64)
    w = 2.0 * np.pi * (f + 0.5) / (2 * T)
    t = np.arange(T, dtype=np.float64)
    ang = w[:, None] * t[None, :]
    fwd = np.concatenate([np.cos(ang), -np.sin(ang)], axis=0)
    inv = np.concatenate([np.cos(ang).T, -np.sin(ang).T], axis=1) / T
    return fwd.astype(np.float32), inv.astype(np.float32)


def _spread(n_items, n_slots):
    return [n_items * (k + 1) // n_slots - n_items * k // n_slots for k in range(n_slots)]


def _interleave(main, side):
    main = list(main)
    cnt = _spread(len(side), len(main))
    it = iter(side)
    for step, c in zip(main, cnt):
        step()
        for _ in range(c):
            next(it)()


def _kernel(zs_ref, q_hbm, k_hbm, v_hbm, shk_hbm, K_hbm, D_hbm, wg_hbm, wu_hbm, wd_hbm, c_hbm, wm_hbm,
            F_hbm, G_hbm, out_hbm,
            kb, vb, Kb, qb, wg, wu, wd, wm, Fm, Gm, shk, Dv, cv, wt, kf, xh0, xh1, y, mod, h2, x1, act,
            ost, sems, osems):
    n_sem = [0]

    def copy(src, dst):
        c = pltpu.make_async_copy(src, dst, sems.at[n_sem[0]])
        n_sem[0] += 1
        return c

    small = [copy(shk_hbm, shk), copy(F_hbm, Fm), copy(D_hbm, Dv), copy(G_hbm, Gm), copy(c_hbm, cv)]
    cp_ct = []
    for ct in range(CT):
        cols = pl.ds(ct * 128, 128)
        cp_ct.append([copy(k_hbm.at[:, cols], kb.at[ct]), copy(v_hbm.at[:, cols], vb.at[ct]),
                      copy(K_hbm.at[cols, :], Kb.at[cols, :])])
    cp_wm = [copy(wm_hbm.at[:, pl.ds(j * D, D)], wm.at[:, pl.ds(j * D, D)]) for j in range(6)]
    q_sem0 = n_sem[0]
    cp_q = [copy(q_hbm.at[pl.ds(min(r, NSTEP - 1) * BM, BM), :], qb.at[r]) for r in range(NSTEP + 1)]
    WC = 256
    cp_wg = [copy(wg_hbm.at[:, pl.ds(j * WC, WC)], wg.at[:, pl.ds(j * WC, WC)]) for j in range(F // WC)]
    cp_wu = [copy(wu_hbm.at[:, pl.ds(j * WC, WC)], wu.at[:, pl.ds(j * WC, WC)]) for j in range(F // WC)]
    cp_wd = [copy(wd_hbm.at[:, pl.ds(j * 128, 128)], wd.at[:, pl.ds(j * 128, 128)]) for j in range(CT)]

    for c in small[:2] + cp_ct[0] + small[2:]:
        c.start()
    for ct in range(1, CT):
        for c in cp_ct[ct]:
            c.start()
    for j in range(5):
        cp_wm[j].start()
    cp_q[0].start()
    for j in range(F // WC):
        cp_wg[j].start()
        cp_wu[j].start()
        if j == 0:
            cp_q[1].start()
    for j in range(CT):
        cp_wd[j].start()
        if j == 0:
            cp_wm[5].start()
    for r in range(2, NSTEP + 1):
        cp_q[r].start()

    zs = zs_ref[0]
    xh = [xh0, xh1]

    kf[pl.ds(0, 8), :] = jnp.zeros((8, 128), F32)
    small[0].wait()
    wt[...] = shk[...].astype(F32)
    small[1].wait()

    def t_stage(ct):
        buf = xh[ct % 2]
        lanes = pl.ds(ct * 128, 128)
        pieces = []

        def wait():
            for c in cp_ct[ct]:
                c.wait()
            if ct == 0:
                small[2].wait()
        pieces.append(wait)

        def unpack(j):
            def run():
                kf[pl.ds(8 + j * T, T), :] = kb[ct, pl.ds(j * T, T), :].astype(F32)
            return run

        def xform(j):
            def run():
                acc = None
                for t in range(4):
                    term = kf[pl.ds(8 + j * T - t, T), :] * wt[pl.ds(t, 1), lanes]
                    acc = term if acc is None else acc + term
                kv = (acc * vb[ct, pl.ds(j * T, T), :].astype(F32)).astype(BF)
                X = jnp.dot(Fm[...], kv, preferred_element_type=F32)
                xr = X[:T].reshape(16, 8, 128)
                xi = X[T:].reshape(16, 8, 128)
                buf[:, 0, j] = xr + xi
                buf[:, 1, j] = xr
                buf[:, 2, j] = xi
            return run

        def hform(j):
            def run():
                H = lax.dot_general(Fm[...], Kb[lanes, pl.ds(j * T, T)], (((1,), (1,)), ((), ())),
                                    preferred_element_type=F32)
                hr = H[:T].reshape(16, 8, 128)
                hi = H[T:].reshape(16, 8, 128)
                if j == 0:
                    hr = hr + Dv[pl.ds(ct, 1), :].astype(F32)
                buf[:, 3, j] = hr
                buf[:, 4, j] = hi - hr
                buf[:, 5, j] = hr + hi
            return run

        pieces.append(unpack(0))
        for j in range(NB):
            if j + 1 < NB:
                pieces.append(unpack(j + 1))
            pieces.append(hform(j))
            pieces.append(xform(j))
        return pieces

    def i_stage(ct):
        buf = xh[ct % 2]
        pieces = []

        def inv(b):
            def run():
                z = jnp.concatenate([buf[:, 6, b].reshape(T, 128), buf[:, 7, b].reshape(T, 128)], axis=0)
                y[pl.ds(b * T, T), pl.ds(ct * 128, 128)] = jnp.dot(Gm[...], z.astype(BF),
                                                                   preferred_element_type=F32)
            return run
        for b in range(NB):
            pieces.append(inv(b))
        return pieces

    def c_stage(ct, G=4, L=3):
        buf = xh[ct % 2]
        steps = []
        for fg in range(16):
            for b0 in range(0, NB, G):
                for m in range(b0 + G - 1, -1, -1):
                    steps.append((fg, b0, m, m == 0))
        loaded, acc, prev = {}, {}, [None]

        def loads_for(si):
            if si >= len(steps):
                return
            fg, b0, m, _ = steps[si]
            loaded[(si, 'h')] = [buf[fg, 3 + p, m] for p in range(3)]
            for b in range(b0, b0 + G):
                i = b - m
                if i >= 0 and (fg, b0, i) not in loaded:
                    loaded[(fg, b0, i)] = [buf[fg, p, i] for p in range(3)]

        def step(si):
            def run():
                if si == 0:
                    for s0 in range(L):
                        loads_for(s0)
                fg, b0, m, last = steps[si]
                loads_for(si + L)
                hs = loaded.pop((si, 'h'))
                for b in range(b0, b0 + G):
                    i = b - m
                    if i < 0:
                        continue
                    x = loaded[(fg, b0, i)]
                    a = acc.setdefault(b, [None, None, None])
                    for p in range(3):
                        t = x[p] * hs[p]
                        a[p] = t if a[p] is None else a[p] + t
                if last:
                    if b0 == 0:
                        prev[0] = None
                    for b in range(b0, b0 + G):
                        a = acc.pop(b)
                        zr, zi = a[0] - a[2], a[0] + a[1]
                        if prev[0] is None:
                            zr2, zi2 = zr, zi
                        elif fg < 8:
                            zr2, zi2 = zr - prev[0][1], zi + prev[0][0]
                        else:
                            zr2, zi2 = zr + prev[0][1], zi - prev[0][0]
                        prev[0] = (zr, zi)
                        buf[zs + fg, 6, b] = zr2
                        buf[zs + fg, 7, b] = zi2
                    for i in range(b0 + G):
                        loaded.pop((fg, b0, i), None)
            return run
        return [step(si) for si in range(len(steps))]

    def mod_piece(j):
        def run():
            if j == 0:
                small[4].wait()
            cp_wm[j].wait()
            cf = cv[...].astype(F32)
            sc = (cf * jax.nn.sigmoid(cf)).astype(BF)
            m = jnp.dot(jnp.broadcast_to(sc, (16, D)), wm[:, pl.ds(j * D, D)], preferred_element_type=F32)
            if j in (1, 4):
                m = m + 1.0
            mod[:, pl.ds(j * D, D)] = m
        return run

    def prep_piece(r, slot, i):
        def run():
            rows = pl.ds(i * 16, 16)
            x = qb[r, rows, :].astype(F32)
            yrows = pl.ds(pl.multiple_of(jnp.minimum(r, NSTEP - 1) * BM + i * 16, 16), 16)
            xc = x - jnp.sum(x, axis=-1, keepdims=True) * (1.0 / D)
            var = jnp.sum(xc * xc, axis=-1, keepdims=True) * (1.0 / D)
            h = xc * lax.rsqrt(var + EPS) * mod[:, pl.ds(D, D)] + mod[:, pl.ds(0, D)]
            xn = x + mod[:, pl.ds(2 * D, D)] * (h * y[yrows, :])
            x1[slot, rows, :] = xn
            xc = xn - jnp.sum(xn, axis=-1, keepdims=True) * (1.0 / D)
            var = jnp.sum(xc * xc, axis=-1, keepdims=True) * (1.0 / D)
            hh = xc * lax.rsqrt(var + EPS) * mod[:, pl.ds(4 * D, D)] + mod[:, pl.ds(3 * D, D)]
            h2[slot, rows, :] = hh.astype(BF)
        return run

    for p in t_stage(0):
        p()
    for ct in range(CT):
        side = []
        if ct + 1 < CT:
            side.append(t_stage(ct + 1))
        if ct >= 1:
            ist = i_stage(ct - 1)
            if ct == 1:
                ist = [small[3].wait] + ist
            side.append(ist)
        if ct == CT - 1:
            side.append([mod_piece(j) for j in range(5)])
        merged = []
        n = max([len(s) for s in side] + [1])
        for kk in range(n):
            for s in side:
                lo, hi = len(s) * kk // n, len(s) * (kk + 1) // n
                merged.extend(s[lo:hi])
        _interleave(c_stage(ct), merged)

    ist = i_stage(CT - 1)
    ist[0]()
    ist[1]()
    cp_q[0].wait()
    _interleave(ist[2:], [prep_piece(0, 0, i) for i in range(BM // 16)])

    def mlp_step(r, slot, first):
        pieces = []

        def gate_up(j):
            def run():
                cols = pl.ds(j * 128, 128)
                if first and j % (WC // 128) == 0:
                    cp_wg[j * 128 // WC].wait()
                    cp_wu[j * 128 // WC].wait()
                h = h2[slot]
                g = jnp.dot(h, wg[:, cols], preferred_element_type=F32)
                u = jnp.dot(h, wu[:, cols], preferred_element_type=F32)
                act[:, cols] = (g * u).astype(BF)
            return run

        def down(n):
            def run():
                cols = pl.ds(n * 128, 128)
                if first:
                    cp_wd[n].wait()
                    if n == 0:
                        mod_piece(5)()
                o = jnp.dot(act[...], wd[:, cols], preferred_element_type=F32)
                gb = mod[:, pl.ds(5 * D + n * 128, 128)]
                gb = jnp.broadcast_to(gb[None], (BM // 16, 16, 128)).reshape(BM, 128)
                ost[r, :, cols] = (x1[slot, :, cols] + gb * o).astype(BF)
            return run
        pieces = [gate_up(j) for j in range(F // 128)] + [down(n) for n in range(CT)]

        def q_wait():
            pltpu.make_async_copy(q_hbm.at[pl.ds(0, BM), :], qb.at[r + 1], sems.at[q_sem0 + r + 1]).wait()
        nxt = [prep_piece(r + 1, 1 - slot, i) for i in range(BM // 16)]
        pieces[0]()
        q_wait()
        _interleave(pieces[1:], nxt)
        pltpu.make_async_copy(ost.at[r], out_hbm.at[pl.ds(r * BM, BM), :], osems.at[r]).start()

    mlp_step(0, 0, True)

    def body(r, carry):
        mlp_step(r, r % 2, False)
        return carry
    lax.fori_loop(1, NSTEP, body, 0)

    for r in range(NSTEP):
        pltpu.make_async_copy(ost.at[r], out_hbm.at[pl.ds(r * BM, BM), :], osems.at[r]).wait()


@jax.jit
def pallas_adaLN_cond__ssm_conv_h3__glu_gated_bilinear__prompt_kernel(
    A_q: jax.Array,
    A_k: jax.Array,
    A_v: jax.Array,
    A_shift_k: jax.Array,
    A_ssm_k: jax.Array,
    A_ssm_D: jax.Array,
    B_x: jax.Array,
    B_w_gate: jax.Array,
    B_w_up: jax.Array,
    B_w_down: jax.Array,
    c: jax.Array,
    w_mod: jax.Array,
):
    del B_x
    fwd, inv = _dft_matrices()
    anyspec = pl.BlockSpec(memory_space=pl.ANY)
    n_sems = 5 + 3 * CT + 6 + (NSTEP + 1) + 2 * (F // 256) + CT
    out = pl.pallas_call(
        _kernel,
        out_shape=jax.ShapeDtypeStruct((S, D), BF),
        in_specs=[pl.BlockSpec(memory_space=pltpu.SMEM)] + [anyspec] * 13,
        out_specs=anyspec,
        scratch_shapes=[
            pltpu.VMEM((CT, S, 128), BF),
            pltpu.VMEM((CT, S, 128), BF),
            pltpu.VMEM((D, S), BF),
            pltpu.VMEM((NSTEP + 1, BM, D), BF),
            pltpu.VMEM((D, F), BF),
            pltpu.VMEM((D, F), BF),
            pltpu.VMEM((F, D), BF),
            pltpu.VMEM((D, 6 * D), BF),
            pltpu.VMEM((2 * T, T), BF),
            pltpu.VMEM((T, 2 * T), BF),
            pltpu.VMEM((4, D), BF),
            pltpu.VMEM((CT, 128), BF),
            pltpu.VMEM((1, D), BF),
            pltpu.VMEM((4, D), F32),
            pltpu.VMEM((8 + S, 128), F32),
            pltpu.VMEM((16, 8, NB, 8, 128), F32),
            pltpu.VMEM((16, 8, NB, 8, 128), F32),
            pltpu.VMEM((S, D), F32),
            pltpu.VMEM((16, 6 * D), F32),
            pltpu.VMEM((2, BM, D), BF),
            pltpu.VMEM((2, BM, D), F32),
            pltpu.VMEM((BM, F), BF),
            pltpu.VMEM((NSTEP, BM, D), BF),
            pltpu.SemaphoreType.DMA((n_sems,)),
            pltpu.SemaphoreType.DMA((NSTEP,)),
        ],
        compiler_params=pltpu.CompilerParams(vmem_limit_bytes=100 * 2**20),
    )(
        np.zeros((1,), np.int32),
        A_q.reshape(S, D), A_k.reshape(S, D), A_v.reshape(S, D), A_shift_k.T, A_ssm_k,
        A_ssm_D.reshape(CT, 128), B_w_gate, B_w_up, B_w_down, c, w_mod,
        jnp.asarray(fwd, BF), jnp.asarray(inv, BF),
    )
    return out.reshape(1, S, D)
```

```python
import numpy as np
import jax
import jax.numpy as jnp
from jax import lax
import jax.experimental.pallas as pl
import jax.experimental.pallas.tpu as pltpu

S, D, F = 2048, 640, 1536
T = 128
NB = S // T
CT = D // 128
BM = 256
NSTEP = S // BM
EPS = 1e-5
BF = jnp.bfloat16
F32 = jnp.float32
P = dict(L=4, HP=5, NC=256, TAIL=1, UO=1)


def _dft_matrices():
    f = np.concatenate([np.arange(0, T, 2), np.arange(1, T, 2)]).astype(np.float64)
    w = 2.0 * np.pi * (f + 0.5) / (2 * T)
    t = np.arange(T, dtype=np.float64)
    ang = w[:, None] * t[None, :]
    fr, fi = np.cos(ang), -np.sin(ang)
    fx = np.stack([fr.reshape(16, 8, T), fi.reshape(16, 8, T)], axis=1).reshape(2 * T, T)
    fh = np.concatenate([fr, fi - fr, fr + fi], axis=0)
    inv = np.concatenate([np.cos(ang).T, -np.sin(ang).T], axis=1) / T
    return fx.astype(np.float32), fh.astype(np.float32), inv.astype(np.float32)


def _pack_rows(a):
    u = a.astype(jnp.bfloat16).view(np.uint16).astype(np.uint32)
    return u[0::2] | (u[1::2] << 16)


def _spread(n_items, n_slots):
    return [n_items * (k + 1) // n_slots - n_items * k // n_slots for k in range(n_slots)]


def _interleave(main, side):
    main = list(main)
    cnt = _spread(len(side), len(main))
    it = iter(side)
    for step, c in zip(main, cnt):
        step()
        for _ in range(c):
            next(it)()


def _kernel(zs_ref, q_hbm, k_hbm, v_hbm, shk_hbm, K_hbm, D_hbm, wg_hbm, wu_hbm, wd_hbm, c_hbm, wm_hbm,
            Fx_hbm, G_hbm, out_hbm,
            kb, vb, Kb, qb, wg, wu, wd, wm, Fx, Gm, shk, Dv, cv, wt, kf, xh, buf, dvf, scv, h2, x1, act,
            ost, sems, osems):
    n_sem = [0]

    def copy(src, dst):
        c = pltpu.make_async_copy(src, dst, sems.at[n_sem[0]])
        n_sem[0] += 1
        return c

    small = [copy(shk_hbm, shk), None, copy(D_hbm, Dv), copy(G_hbm, Gm), copy(c_hbm, cv), copy(Fx_hbm, Fx)]
    ct_sem0 = n_sem[0]
    cp_ct = []
    for ct in range(CT):
        cols = pl.ds(ct * 128, 128)
        cp_ct.append([copy(k_hbm.at[:, cols], kb.at[ct]), copy(v_hbm.at[:, cols], vb.at[ct]),
                      copy(K_hbm.at[cols, :], Kb.at[cols, :])])
    wm_sem0 = n_sem[0]
    cp_wm = [copy(wm_hbm.at[:, pl.ds(j * D, D)], wm.at[:, pl.ds(j * D, D)]) for j in range(6)]
    q_sem0 = n_sem[0]
    cp_q = [copy(q_hbm.at[pl.ds(min(r, NSTEP - 1) * BM, BM), :], qb.at[r]) for r in range(NSTEP)]
    WC = 256
    cp_wg = [copy(wg_hbm.at[:, pl.ds(j * WC, WC)], wg.at[:, pl.ds(j * WC, WC)]) for j in range(F // WC)]
    cp_wu = [copy(wu_hbm.at[:, pl.ds(j * WC, WC)], wu.at[:, pl.ds(j * WC, WC)]) for j in range(F // WC)]
    cp_wd = [copy(wd_hbm.at[:, pl.ds(j * 128, 128)], wd.at[:, pl.ds(j * 128, 128)]) for j in range(CT)]

    for c in [small[0], small[5], small[2], small[4]] + cp_ct[0] + [small[3], cp_wm[0]]:
        c.start()
    for ct in range(1, CT):
        for c in cp_ct[ct]:
            c.start()
        cp_wm[ct].start()
    cp_q[0].start()
    for j in range(F // WC):
        cp_wg[j].start()
        cp_wu[j].start()
    cp_q[1].start()
    for j in range(CT):
        cp_wd[j].start()
    cp_wm[5].start()
    for r in range(2, NSTEP):
        cp_q[r].start()

    zs = zs_ref[0]
    n_blk = [0]

    def block(fn):
        n_blk[0] += 1
        pl.when(zs_ref[n_blk[0]] == 0)(fn)

    small[0].wait()
    wt[...] = shk[...].astype(F32)
    small[5].wait()
    kf[pl.ds(0, 8), :] = jnp.zeros((8, 128), F32)

    def kv_block(ct, j):
        rows = pl.ds(j * T, T)
        lanes = pl.ds(pl.multiple_of(ct * 128, 128), 128)
        acc = None
        for t in range(4):
            term = kf[pl.ds(8 + j * T - t, T), :] * wt[pl.ds(t, 1), lanes]
            acc = term if acc is None else acc + term
        return (acc * vb[ct, rows, :].astype(F32)).astype(BF)

    def unpack(ct, j):
        kf[pl.ds(8 + j * T, T), :] = kb[ct, pl.ds(j * T, T), :].astype(F32)

    def xform(ct, j):
        v = jnp.dot(pltpu.bitcast(Fx[...], BF), kv_block(ct, j), preferred_element_type=F32).reshape(16, 2, 8, 128)
        re, im = v[:, 0], v[:, 1]
        xh[:, 0, j] = re + im
        xh[:, 1, j] = re
        xh[:, 2, j] = im

    def hform(ct, j):
        H = lax.dot_general(pltpu.bitcast(Fx[...], BF), Kb[pl.ds(pl.multiple_of(ct * 128, 128), 128), pl.ds(j * T, T)],
                            (((1,), (1,)), ((), ())), preferred_element_type=F32).reshape(16, 2, 8, 128)
        re, im = H[:, 0], H[:, 1]
        if j == 0:
            re = re + dvf[ct]
        xh[:, 3, j] = re
        xh[:, 4, j] = im - re
        xh[:, 5, j] = re + im

    def inv(ct, b):
        g = pltpu.bitcast(Gm[...], BF)
        z = [jnp.concatenate([pltpu.bitcast(xh[fg, p, b], BF) for fg in range(1, 16, 2)], axis=0) for p in (6, 7)]
        yb = jnp.dot(g, jnp.concatenate(z, axis=0), preferred_element_type=F32)
        buf[:, ct, b] = yb.reshape(16, 8, 128)

    def conv(ct, G=4, L=P['L']):
        steps = []
        for b0 in range(0, NB, G):
            for fg in range(16):
                for m in range(b0 + G - 1, -1, -1):
                    steps.append((fg, b0, m, m == 0))
        loaded, acc, even = {}, {}, {}

        def loads_for(si):
            if si >= len(steps):
                return
            fg, b0, m, last = steps[si]
            loaded[(si, 'h')] = [xh[fg, 3 + p, m] for p in range(3)]
            for b in range(b0, b0 + G):
                i = b - m
                if i >= 0 and (fg, b0, i) not in loaded:
                    loaded[(fg, b0, i)] = [xh[fg, p, i] for p in range(3)]
            if last and b0 > 0:
                loaded[(fg, b0, 'prev')] = (xh[fg, 8, 0], xh[fg, 8, 1])

        for s0 in range(L):
            loads_for(s0)
        for si, (fg, b0, m, last) in enumerate(steps):
            if b0 > 0 and fg % 4 == 0 and m == b0 + G - 1 - P['HP']:
                inv(ct, b0 - G + fg // 4)
            loads_for(si + L)
            hs = loaded.pop((si, 'h'))
            for b in range(b0, b0 + G):
                i = b - m
                if i < 0:
                    continue
                x = loaded[(fg, b0, i)]
                a = acc.setdefault(b, [None, None, None])
                for p in range(3):
                    t = x[p] * hs[p]
                    a[p] = t if a[p] is None else a[p] + t
            if last:
                prev = loaded.pop((fg, b0, 'prev'), None)
                for b in range(b0, b0 + G):
                    a = acc.pop(b)
                    zr, zi = a[0] - a[2], a[0] + a[1]
                    if prev is None:
                        zr2, zi2 = zr, zi
                    elif fg < 8:
                        zr2, zi2 = zr - prev[1], zi + prev[0]
                    else:
                        zr2, zi2 = zr + prev[1], zi - prev[0]
                    prev = (zr, zi)
                    if fg % 2 == 0:
                        even[b] = (zr2, zi2)
                    else:
                        er, ei = even.pop(b)
                        xh[zs + fg, 6, b] = pltpu.bitcast(jnp.concatenate([er, zr2], axis=0).astype(BF), F32)
                        xh[zs + fg, 7, b] = pltpu.bitcast(jnp.concatenate([ei, zi2], axis=0).astype(BF), F32)
                if b0 + G < NB:
                    xh[zs + fg, 8, 0] = prev[0]
                    xh[zs + fg, 8, 1] = prev[1]
        for b in range(NB - G, NB):
            inv(ct, b)

    def mod_piece(j):
        cols = pl.ds(pl.multiple_of(j * D, 128), D)
        pltpu.make_async_copy(wm_hbm.at[:, cols], wm.at[:, cols], sems.at[wm_sem0 + j]).wait()
        m = jnp.dot(scv[...], wm[:, cols], preferred_element_type=F32)
        m = m + jnp.where((j == 1) | (j == 4), 1.0, 0.0)
        for n in range(CT):
            buf[0:2, 5 + j % 3, (j // 3) * CT + n] = m[:, n * 128:(n + 1) * 128].reshape(2, 8, 128)

    def modv(j, n=None):
        if n is not None:
            return buf[0:2, 5 + j % 3, (j // 3) * CT + n].reshape(16, 128)
        v = jnp.concatenate([buf[0, 5 + j % 3, (j // 3) * CT + n] for n in range(CT)], axis=1)
        return jnp.concatenate([v, v], axis=0)

    def prep_piece(r, slot, i):
        def run():
            rows = pl.ds(i * 16, 16)
            x = qb[r, rows, :].astype(F32)
            yb = jnp.minimum(r, NSTEP - 1) * (BM // T) + i // 8
            yv = jnp.concatenate([buf[pl.ds((i % 8) * 2, 2), n, yb].reshape(16, 128) for n in range(CT)], axis=1)
            xc = x - jnp.sum(x, axis=-1, keepdims=True) * (1.0 / D)
            var = jnp.sum(xc * xc, axis=-1, keepdims=True) * (1.0 / D)
            h = xc * lax.rsqrt(var + EPS) * modv(1) + modv(0)
            xn = x + modv(2) * (h * yv)
            x1[slot, rows, :] = xn
            xc = xn - jnp.sum(xn, axis=-1, keepdims=True) * (1.0 / D)
            var = jnp.sum(xc * xc, axis=-1, keepdims=True) * (1.0 / D)
            hh = xc * lax.rsqrt(var + EPS) * modv(4) + modv(3)
            h2[slot, rows, :] = hh.astype(BF)
        return run

    small[2].wait()
    for ct in range(CT):
        dvf[ct] = Dv[pl.ds(ct, 1), :].astype(F32)
    small[4].wait()
    cf = cv[...].astype(F32)
    scv[...] = jnp.broadcast_to((cf * jax.nn.sigmoid(cf)).astype(BF), (16, D))
    small[3].wait()

    def ct_body(ct, carry):
        for e, (src, dst) in enumerate([(k_hbm.at[:, pl.ds(0, 128)], kb.at[0]), (v_hbm.at[:, pl.ds(0, 128)], vb.at[0]),
                                        (K_hbm.at[pl.ds(0, 128), :], Kb.at[pl.ds(0, 128), :])]):
            pltpu.make_async_copy(src, dst, sems.at[ct_sem0 + 3 * ct + e]).wait()
        for j in range(P['UO']):
            unpack(ct, j)
        for j in range(NB):
            if j + P['UO'] < NB:
                unpack(ct, j + P['UO'])
            hform(ct, j)
            xform(ct, j)
        mod_piece(ct)
        conv(ct)
        return carry
    lax.fori_loop(0, CT, ct_body, 0)

    cp_q[0].wait()
    for i in range(BM // 16):
        prep_piece(0, 0, i)()

    def mlp_step(r, slot, first, last=False):
        pieces = []

        def gate_up(j):
            def run():
                cols = pl.ds(j * P['NC'], P['NC'])
                h = h2[slot]
                g = jnp.dot(h, wg[:, cols], preferred_element_type=F32)
                u = jnp.dot(h, wu[:, cols], preferred_element_type=F32)
                act[:, cols] = (g * u).astype(BF)
            return run

        def tail(n):
            cols = pl.ds(n * 128, 128)
            return pltpu.make_async_copy(ost.at[r, :, cols], out_hbm.at[pl.ds(r * BM, BM), cols], osems.at[r + n])

        def down(n):
            def run():
                cols = pl.ds(n * 128, 128)
                if first and n == 0:
                    for c in cp_wd:
                        c.wait()
                    mod_piece(5)
                o = jnp.dot(act[...], wd[:, cols], preferred_element_type=F32)
                gb = modv(5, n)
                gb = jnp.broadcast_to(gb[None], (BM // 16, 16, 128)).reshape(BM, 128)
                ost[r, :, cols] = (x1[slot, :, cols] + gb * o).astype(BF)
                if last and P['TAIL']:
                    tail(n).start()
            return run
        pieces = [gate_up(j) for j in range(F // P['NC'])] + [down(n) for n in range(CT)]

        def q_wait():
            pltpu.make_async_copy(q_hbm.at[pl.ds(0, BM), :], qb.at[r + 1], sems.at[q_sem0 + r + 1]).wait()
        nxt = [prep_piece(r + 1, 1 - slot, i) for i in range(BM // 16)]
        if first:
            for c in cp_wg + cp_wu + [cp_q[1]]:
                c.wait()
        if last:
            nxt = []
        _interleave(pieces, nxt)
        if last and P['TAIL']:
            for n in range(CT):
                tail(n).wait()
        else:
            pltpu.make_async_copy(ost.at[r], out_hbm.at[pl.ds(r * BM, BM), :], osems.at[r]).start()

    mlp_step(0, 0, True)

    for c in cp_q[2:]:
        c.wait()

    def body(r, carry):
        mlp_step(r, r % 2, False)
        return carry
    lax.fori_loop(1, NSTEP - 1, body, 0)
    mlp_step(NSTEP - 1, 1, False, True)

    for r in range(NSTEP - P['TAIL']):
        pltpu.make_async_copy(ost.at[r], out_hbm.at[pl.ds(r * BM, BM), :], osems.at[r]).wait()


@jax.jit
def pallas_adaLN_cond__ssm_conv_h3__glu_gated_bilinear__prompt_kernel(
    A_q: jax.Array,
    A_k: jax.Array,
    A_v: jax.Array,
    A_shift_k: jax.Array,
    A_ssm_k: jax.Array,
    A_ssm_D: jax.Array,
    B_x: jax.Array,
    B_w_gate: jax.Array,
    B_w_up: jax.Array,
    B_w_down: jax.Array,
    c: jax.Array,
    w_mod: jax.Array,
):
    del B_x
    fx, fh, inv = _dft_matrices()
    anyspec = pl.BlockSpec(memory_space=pl.ANY)
    n_sems = 5 + 3 * CT + 6 + NSTEP + 2 * (F // 256) + CT
    out = pl.pallas_call(
        _kernel,
        out_shape=jax.ShapeDtypeStruct((S, D), BF),
        in_specs=[pl.BlockSpec(memory_space=pltpu.SMEM)] + [anyspec] * 13,
        out_specs=anyspec,
        scratch_shapes=[
            pltpu.VMEM((CT, S, 128), BF),
            pltpu.VMEM((CT, S, 128), BF),
            pltpu.VMEM((D, S), BF),
            pltpu.VMEM((NSTEP, BM, D), BF),
            pltpu.VMEM((D, F), BF),
            pltpu.VMEM((D, F), BF),
            pltpu.VMEM((F, D), BF),
            pltpu.VMEM((D, 6 * D), BF),
            pltpu.VMEM((T, T), jnp.uint32),
            pltpu.VMEM((T // 2, 2 * T), jnp.uint32),
            pltpu.VMEM((4, D), BF),
            pltpu.VMEM((CT, 128), BF),
            pltpu.VMEM((1, D), BF),
            pltpu.VMEM((4, D), F32),
            pltpu.VMEM((8 + S, 128), F32),
            pltpu.VMEM((16, 9, NB, 8, 128), F32),
            pltpu.VMEM((16, 8, NB, 8, 128), F32),
            pltpu.VMEM((CT, 1, 128), F32),
            pltpu.VMEM((16, D), BF),
            pltpu.VMEM((2, BM, D), BF),
            pltpu.VMEM((2, BM, D), F32),
            pltpu.VMEM((BM, F), BF),
            pltpu.VMEM((NSTEP, BM, D), BF),
            pltpu.SemaphoreType.DMA((n_sems,)),
            pltpu.SemaphoreType.DMA((NSTEP + CT,)),
        ],
        compiler_params=pltpu.CompilerParams(vmem_limit_bytes=100 * 2**20),
    )(
        np.zeros((1,), np.int32),
        A_q.reshape(S, D), A_k.reshape(S, D), A_v.reshape(S, D), A_shift_k.T, A_ssm_k,
        A_ssm_D.reshape(CT, 128), B_w_gate, B_w_up, B_w_down, c, w_mod,
        _pack_rows(fx), _pack_rows(inv),
    )
    return out.reshape(1, S, D)
```
